```python
import os as _os
_os.environ.setdefault("JAX_PLATFORMS", "cpu")
import jax
import jax.numpy as jnp

def _softmax(x, axis=-1):
    return jax.nn.softmax(x, axis=axis)
def _gelu(x):
    return jax.nn.gelu(x, approximate=True)
def _silu(x):
    return jax.nn.silu(x)
def _sigmoid(x):
    return jax.nn.sigmoid(x)
def _layernorm(x, axis=-1, eps=1e-5):
    m = jnp.mean(x, axis=axis, keepdims=True)
    v = jnp.var(x, axis=axis, keepdims=True)
    return (x - m) / jnp.sqrt(v + eps)
def _scatter_add(tgt, idx, src, axis=0):
    return tgt.at[idx].add(src)
def _segment_sum(src, seg, n):
    return jax.ops.segment_sum(src, seg, n)
class _Rng:
    def __init__(self, key):
        self._k = key
    def _next(self):
        self._k, sub = jax.random.split(self._k)
        return sub
    def normal(self, shape):
        return jax.random.normal(self._next(), shape, dtype=jnp.bfloat16)
    def randint(self, lo, hi, shape):
        return jax.random.randint(self._next(), shape, lo, hi, dtype=jnp.int32)
    def uniform(self, shape, lo=0.0, hi=1.0):
        return jax.random.uniform(self._next(), shape, jnp.bfloat16, lo, hi)
    def permutation(self, n):
        return jax.random.permutation(self._next(), n)


kernel_name = 'sequential_preLN__sliding_local_dilated__dense_activation_relu__prompt'

def setup_inputs():
    _rng = _Rng(jax.random.key(int.from_bytes(__import__("os").urandom(4), "little")))
    _w = (lambda a: (lambda t: t.astype(jnp.bfloat16) if jnp.issubdtype(t.dtype, jnp.floating) else t)(jnp.asarray(a)))
    def _A_setup():
        B, S, D = 1, 2048, 1024
        return {
            "x": _w((lambda *s: _rng.normal(s) * 0.05)(B, S, D)),
            "wqkv": _w((lambda *s: _rng.normal(s) * 0.05)(D, 3 * D)),
            "wo": _w((lambda *s: _rng.normal(s) * 0.05)(D, D)),
        }
    _A_in = _A_setup()

    def _B_setup():
        B, S, D, Dff = 1, 2048, 1024, 3584
        return {
            "x": _w((lambda *s: _rng.normal(s) * 0.05)(B, S, D)),
            "w1": _w((lambda *s: _rng.normal(s) * 0.05)(D, Dff)),
            "w2": _w((lambda *s: _rng.normal(s) * 0.05)(Dff, D)),
        }
    _B_in = _B_setup()

    return {
        "A_x": _A_in["x"],
        "A_wqkv": _A_in["wqkv"],
        "A_wo": _A_in["wo"],
        "B_x": _B_in["x"],
        "B_w1": _B_in["w1"],
        "B_w2": _B_in["w2"],
    }

def reference(A_x, A_wqkv, A_wo, B_x, B_w1, B_w2):
    def _A_ref(x, wqkv, wo):
        B, S, D = x.shape
        H = 32; Dh = D // H
        W, dil = 8, 2
        qkv = (lambda x, *d: x.transpose(*d))((x @ wqkv).reshape(B, S, 3, H, Dh), 2, 0, 3, 1, 4)
        q, k, v = qkv[0], qkv[1], qkv[2]
        scale = Dh ** -0.5
        pos = jnp.arange(S)
        off = jnp.arange(W) * dil
        idx = pos[:, None] - off[None, :]
        mask = idx >= 0
        idx_c = jnp.where(mask, idx, 0).reshape(-1)
        kg = k[:, :, idx_c, :].reshape(B, H, S, W, Dh)
        vg = v[:, :, idx_c, :].reshape(B, H, S, W, Dh)
        logits = jnp.einsum("bhsd,bhswd->bhsw", q, kg) * scale
        logits = jnp.where(mask[None, None, :, :], logits, -1e9)
        attn = _softmax(logits, axis=-1)
        o = jnp.einsum("bhsw,bhswd->bhsd", attn, vg)
        return (lambda x, *d: x.transpose(*d))(o, 0, 2, 1, 3).reshape(B, S, D) @ wo

    def _B_ref(x, w1, w2):
        h = jnp.einsum("bsd,df->bsf", x, w1)
        zero = jnp.zeros_like(h)
        h = jnp.maximum(h, zero)
        return jnp.einsum("bsf,fd->bsd", h, w2)

    x = A_x
    h = x + _A_ref(_layernorm(x, axis=-1), A_wqkv, A_wo)
    h2 = h + _B_ref(_layernorm(h, axis=-1), B_w1, B_w2)
    return h2
```

```python
import functools
import jax
import jax.numpy as jnp
import jax.experimental.pallas as pl
import jax.experimental.pallas.tpu as pltpu

S, D, H, DH, DFF = 2048, 1024, 32, 32, 3584
W, DIL = 8, 2
HALO = 16
T = 256
R = 16
EPS = 1e-5
SCALE = DH ** -0.5


def _ln(x):
    m = jnp.mean(x, axis=-1, keepdims=True)
    xc = x - m
    v = jnp.mean(xc * xc, axis=-1, keepdims=True)
    return xc * jax.lax.rsqrt(v + EPS)


def _rb(x):
    return x.astype(jnp.bfloat16).astype(jnp.float32)


def kernel(x_ref, wqkv_hbm, wo_hbm, w1_hbm, w2_hbm, o_ref,
           wqkv_v, wo_v, w1_v, w2_v, t1_scr, wo32_scr, q_scr, k_scr, v_scr, oa_scr, sems):
    i = pl.program_id(0)

    @pl.when(i == 0)
    def _prep():
        cq = pltpu.make_async_copy(wqkv_hbm, wqkv_v, sems.at[0])
        co = pltpu.make_async_copy(wo_hbm, wo_v, sems.at[1])
        c1 = pltpu.make_async_copy(w1_hbm, w1_v, sems.at[2])
        c2 = pltpu.make_async_copy(w2_hbm, w2_v, sems.at[3])
        cq.start(); co.start(); c1.start(); c2.start()
        k_scr[0:HALO, :] = jnp.zeros((HALO, D), jnp.float32)
        v_scr[0:HALO, :] = jnp.zeros((HALO, D), jnp.float32)
        cq.wait()
        for m in range(3):
            for cb in range(8):
                blk = wqkv_v[:, m * D + cb * 128: m * D + (cb + 1) * 128]
                u = pltpu.bitcast(blk, jnp.uint32)
                for rb in range(4):
                    t1_scr[rb, cb * 128:(cb + 1) * 128, :] = u[rb * 128:(rb + 1) * 128, :].T
            for cb in range(8):
                for rb in range(4):
                    parts = [t1_scr[rb, pl.ds(cb * 4 + j, 32, stride=32), :] for j in range(4)]
                    g = jnp.concatenate(parts, axis=0)
                    wqkv_v[rb * 256:(rb + 1) * 256, m * D + cb * 128: m * D + (cb + 1) * 128] = pltpu.bitcast(g.T, jnp.bfloat16)
        co.wait()
        for cb in range(8):
            wo32_scr[cb] = wo_v[:, cb * 128:(cb + 1) * 128].astype(jnp.float32)
        for cb in range(8):
            for cj in range(32):
                wo_v[cj * 32:(cj + 1) * 32, cb * 128:(cb + 1) * 128] = wo32_scr[cb, pl.ds(cj, 32, stride=32), :].astype(jnp.bfloat16)
        c1.wait()
        c2.wait()

    x = x_ref[...].astype(jnp.float32)
    xn = _ln(x).astype(jnp.bfloat16)
    q_scr[...] = _rb(jnp.dot(xn, wqkv_v[:, 0:D], preferred_element_type=jnp.float32))
    k_scr[HALO:HALO + T, :] = _rb(jnp.dot(xn, wqkv_v[:, D:2 * D], preferred_element_type=jnp.float32))
    v_scr[HALO:HALO + T, :] = _rb(jnp.dot(xn, wqkv_v[:, 2 * D:3 * D], preferred_element_type=jnp.float32))

    row0 = i * T
    for c in range(T // R):
        r0 = c * R
        q = q_scr[r0:r0 + R, :]
        rows = row0 + r0 + jax.lax.broadcasted_iota(jnp.int32, (R, 128), 0)
        logits = []
        for w in range(W):
            kw = k_scr[r0 + HALO - DIL * w: r0 + HALO - DIL * w + R, :]
            p = q * kw
            s = p[:, 0:128]
            for cb in range(1, 8):
                s = s + p[:, cb * 128:(cb + 1) * 128]
            s = s + pltpu.roll(s, 64, 1)
            s = s + pltpu.roll(s, 32, 1)
            s = s * SCALE
            if w > 0:
                s = jnp.where(rows >= DIL * w, s, -1e9)
            logits.append(s)
        m = logits[0]
        for w in range(1, W):
            m = jnp.maximum(m, logits[w])
        es = [jnp.exp(l - m) for l in logits]
        den = es[0]
        for w in range(1, W):
            den = den + es[w]
        inv = 1.0 / den
        acc = None
        for w in range(W):
            a = es[w] * inv
            a8 = jnp.concatenate([a] * 8, axis=1)
            vw = v_scr[r0 + HALO - DIL * w: r0 + HALO - DIL * w + R, :]
            acc = a8 * vw if acc is None else acc + a8 * vw
        oa_scr[r0:r0 + R, :] = acc.astype(jnp.bfloat16)

    k_scr[0:HALO, :] = k_scr[T:T + HALO, :]
    v_scr[0:HALO, :] = v_scr[T:T + HALO, :]

    ao = jnp.dot(oa_scr[...], wo_v[...], preferred_element_type=jnp.float32)
    h = _rb(x + _rb(ao))
    hn = _ln(h).astype(jnp.bfloat16)
    h1 = jnp.maximum(jnp.dot(hn, w1_v[...], preferred_element_type=jnp.float32), 0.0).astype(jnp.bfloat16)
    y = jnp.dot(h1, w2_v[...], preferred_element_type=jnp.float32)
    o_ref[...] = (h + _rb(y)).astype(jnp.bfloat16)


@jax.jit
def pallas_sequential_preLN__sliding_local_dilated__dense_activation_relu__prompt_kernel(
    A_x, A_wqkv, A_wo, B_x, B_w1, B_w2):
    x = A_x.reshape(S, D)
    out = pl.pallas_call(
        kernel,
        grid=(S // T,),
        in_specs=[
            pl.BlockSpec((T, D), lambda i: (i, 0)),
            pl.BlockSpec(memory_space=pl.ANY),
            pl.BlockSpec(memory_space=pl.ANY),
            pl.BlockSpec(memory_space=pl.ANY),
            pl.BlockSpec(memory_space=pl.ANY),
        ],
        out_specs=pl.BlockSpec((T, D), lambda i: (i, 0)),
        out_shape=jax.ShapeDtypeStruct((S, D), jnp.bfloat16),
        scratch_shapes=[
            pltpu.VMEM((D, 3 * D), jnp.bfloat16),
            pltpu.VMEM((D, D), jnp.bfloat16),
            pltpu.VMEM((D, DFF), jnp.bfloat16),
            pltpu.VMEM((DFF, D), jnp.bfloat16),
            pltpu.VMEM((4, D, 128), jnp.uint32),
            pltpu.VMEM((8, D, 128), jnp.float32),
            pltpu.VMEM((T, D), jnp.float32),
            pltpu.VMEM((T + HALO, D), jnp.float32),
            pltpu.VMEM((T + HALO, D), jnp.float32),
            pltpu.VMEM((T, D), jnp.bfloat16),
            pltpu.SemaphoreType.DMA((4,)),
        ],
        compiler_params=pltpu.CompilerParams(
            dimension_semantics=("arbitrary",),
            vmem_limit_bytes=100 * 1024 * 1024,
        ),
    )(x, A_wqkv, A_wo, B_w1, B_w2)
    return out.reshape(1, S, D)
```

```python
import jax
import jax.numpy as jnp
import jax.experimental.pallas as pl
import jax.experimental.pallas.tpu as pltpu

S, D, H, DH, DFF = 2048, 1024, 32, 32, 3584
W, DIL = 8, 2
HALO = 16
T = 256
N = S // T
R = 64
EPS = 1e-5
SCALE = DH ** -0.5


def _ln(x):
    m = jnp.mean(x, axis=-1, keepdims=True)
    xc = x - m
    v = jnp.mean(xc * xc, axis=-1, keepdims=True)
    return xc * jax.lax.rsqrt(v + EPS)


def _rb(x):
    return x.astype(jnp.bfloat16).astype(jnp.float32)


def _perm_tile(load_tile, a, p, b21, low):
    a0, a21 = a & 1, a >> 1
    t0 = (((b21 * 2 + 0) * 4 + p) * 4) + a21
    t1 = (((b21 * 2 + 1) * 4 + p) * 4) + a21
    x0, x1 = load_tile(t0), load_tile(t1)
    if a0 == 0:
        return jnp.where(low, x0, pltpu.roll(x1, 4, 0))
    return jnp.where(low, pltpu.roll(x0, 4, 0), x1)


def _kernel(x_ref, xnext_ref, wqkv_hbm, wo_hbm, w1_hbm, w2_hbm, o_ref,
            wqkv_v, wo_v, w1_v, w2_v, t1_scr, wo2_v, q_scr, k_scr, v_scr, oa_scr, xn_scr, sems):
    i = pl.program_id(0)

    def cq(m):
        return pltpu.make_async_copy(wqkv_hbm.at[:, pl.ds(m * D, D)], wqkv_v.at[m], sems.at[m])
    co = pltpu.make_async_copy(wo_hbm, wo_v, sems.at[3])
    c1 = pltpu.make_async_copy(w1_hbm, w1_v, sems.at[4])
    c2 = pltpu.make_async_copy(w2_hbm, w2_v, sems.at[5])

    @pl.when(i == 0)
    def _prep():
        cq(0).start()
        cq(1).start()
        cq(2).start()
        k_scr[0:HALO, :] = jnp.zeros((HALO, D), jnp.float32)
        v_scr[0:HALO, :] = jnp.zeros((HALO, D), jnp.float32)
        xn_scr[...] = _ln(x_ref[...].astype(jnp.float32)).astype(jnp.bfloat16)
        low = jax.lax.broadcasted_iota(jnp.int32, (8, 128), 0) < 4
        u = wqkv_v.bitcast(jnp.uint32)
        for m in range(3):
            cq(m).wait()
            if m == 0:
                co.start()
            if m == 2:
                c1.start()
                c2.start()
            for cb in range(8):
                for rb in range(4):
                    t1_scr[rb, cb * 128:(cb + 1) * 128, :] = (
                        u[m, rb * 128:(rb + 1) * 128, cb * 128:(cb + 1) * 128].T)
            for a in range(8):
                for rb in range(4):
                    tiles = [_perm_tile(lambda t: t1_scr[rb, t * 8:(t + 1) * 8, :], a, p, b21, low)
                             for p in range(4) for b21 in range(4)]
                    g = jnp.concatenate(tiles, axis=0)
                    u[m, rb * 128:(rb + 1) * 128, a * 128:(a + 1) * 128] = g.T
        co.wait()
        for cb in range(8):
            for a in range(8):
                for p in range(4):
                    for b2 in range(2):
                        ld = lambda t: wo_v[t * 8:(t + 1) * 8, cb * 128:(cb + 1) * 128].astype(jnp.float32)
                        g = jnp.concatenate(
                            [_perm_tile(ld, a, p, b2 * 2 + b1, low) for b1 in range(2)], axis=0)
                        r0 = a * 128 + p * 32 + b2 * 16
                        wo2_v[r0:r0 + 16, cb * 128:(cb + 1) * 128] = g.astype(jnp.bfloat16)

    xn = xn_scr[...]
    q_scr[...] = _rb(jnp.dot(xn, wqkv_v[0], preferred_element_type=jnp.float32))
    k_scr[HALO:HALO + T, :] = _rb(jnp.dot(xn, wqkv_v[1], preferred_element_type=jnp.float32))
    v_scr[HALO:HALO + T, :] = _rb(jnp.dot(xn, wqkv_v[2], preferred_element_type=jnp.float32))

    lane = jax.lax.broadcasted_iota(jnp.int32, (R, 128), 1)
    even1 = (lane & 1) == 0
    even2 = (lane & 2) == 0
    row0 = i * T
    for c in range(T // R):
        r0 = c * R
        q = q_scr[r0:r0 + R, :]
        logits = []
        ksh = [k_scr[r0 + HALO - 8 - DIL * a: r0 + HALO - DIL * a + R, :] for a in range(4)]
        for w in range(W):
            kw = ksh[w][8:8 + R] if w < 4 else ksh[w - 4][0:R]
            p = q * kw
            s = p[:, 0:128]
            for cb in range(1, 8):
                s = s + p[:, cb * 128:(cb + 1) * 128]
            s = s + jnp.where(even1, pltpu.roll(s, 127, 1), pltpu.roll(s, 1, 1))
            s = s + jnp.where(even2, pltpu.roll(s, 126, 1), pltpu.roll(s, 2, 1))
            s = s * SCALE
            if w > 0 and r0 < DIL * w:
                rows = row0 + r0 + jax.lax.broadcasted_iota(jnp.int32, (R, 128), 0)
                s = jnp.where(rows >= DIL * w, s, -1e9)
            logits.append(s)
        m = logits[0]
        for w in range(1, W):
            m = jnp.maximum(m, logits[w])
        es = [jnp.exp(l - m) for l in logits]
        den = es[0]
        for w in range(1, W):
            den = den + es[w]
        inv = 1.0 / den
        acc = None
        vsh = [v_scr[r0 + HALO - 8 - DIL * a: r0 + HALO - DIL * a + R, :] for a in range(4)]
        for w in range(W):
            a = es[w] * inv
            a8 = jnp.concatenate([a] * 8, axis=1)
            vw = vsh[w][8:8 + R] if w < 4 else vsh[w - 4][0:R]
            acc = a8 * vw if acc is None else acc + a8 * vw
        oa_scr[r0:r0 + R, :] = acc.astype(jnp.bfloat16)

    k_scr[0:HALO, :] = k_scr[T:T + HALO, :]
    v_scr[0:HALO, :] = v_scr[T:T + HALO, :]

    ao = jnp.dot(oa_scr[...], wo2_v[...], preferred_element_type=jnp.float32)
    h = _rb(x_ref[...].astype(jnp.float32) + _rb(ao))
    hn = _ln(h).astype(jnp.bfloat16)
    pl.when(i == 0)(lambda: c1.wait())
    h1 = jnp.maximum(jnp.dot(hn, w1_v[...], preferred_element_type=jnp.float32), 0.0).astype(jnp.bfloat16)
    xn_scr[...] = _ln(xnext_ref[...].astype(jnp.float32)).astype(jnp.bfloat16)
    pl.when(i == 0)(lambda: c2.wait())
    y = jnp.dot(h1, w2_v[...], preferred_element_type=jnp.float32)
    o_ref[...] = (h + _rb(y)).astype(jnp.bfloat16)


@jax.jit
def pallas_sequential_preLN__sliding_local_dilated__dense_activation_relu__prompt_kernel(
    A_x: jax.Array,
    A_wqkv: jax.Array,
    A_wo: jax.Array,
    B_x: jax.Array,
    B_w1: jax.Array,
    B_w2: jax.Array,
):
    x = A_x.reshape(S, D)
    out = pl.pallas_call(
        _kernel,
        grid=(N,),
        in_specs=[
            pl.BlockSpec((T, D), lambda i: (i, 0)),
            pl.BlockSpec((T, D), lambda i: (jnp.minimum(i + 1, N - 1), 0)),
            pl.BlockSpec(memory_space=pl.ANY),
            pl.BlockSpec(memory_space=pl.ANY),
            pl.BlockSpec(memory_space=pl.ANY),
            pl.BlockSpec(memory_space=pl.ANY),
        ],
        out_specs=pl.BlockSpec((T, D), lambda i: (i, 0)),
        out_shape=jax.ShapeDtypeStruct((S, D), jnp.bfloat16),
        scratch_shapes=[
            pltpu.VMEM((3, D, D), jnp.bfloat16),
            pltpu.VMEM((D, D), jnp.bfloat16),
            pltpu.VMEM((D, DFF), jnp.bfloat16),
            pltpu.VMEM((DFF, D), jnp.bfloat16),
            pltpu.VMEM((4, D, 128), jnp.uint32),
            pltpu.VMEM((D, D), jnp.bfloat16),
            pltpu.VMEM((T, D), jnp.float32),
            pltpu.VMEM((T + HALO, D), jnp.float32),
            pltpu.VMEM((T + HALO, D), jnp.float32),
            pltpu.VMEM((T, D), jnp.bfloat16),
            pltpu.VMEM((T, D), jnp.bfloat16),
            pltpu.SemaphoreType.DMA((6,)),
        ],
        compiler_params=pltpu.CompilerParams(
            dimension_semantics=("arbitrary",),
            vmem_limit_bytes=100 * 1024 * 1024,
        ),
    )(x, x, A_wqkv, A_wo, B_w1, B_w2)
    return out.reshape(1, S, D)
```

```python
import jax
import jax.numpy as jnp
import jax.experimental.pallas as pl
import jax.experimental.pallas.tpu as pltpu

S, D, H, DH, DFF = 2048, 1024, 32, 32, 3584
W, DIL = 8, 2
HALO = 16
T = 256
N = S // T
R = 64
EPS = 1e-5
SCALE = DH ** -0.5


def _ln(x):
    m = jnp.mean(x, axis=-1, keepdims=True)
    xc = x - m
    v = jnp.mean(xc * xc, axis=-1, keepdims=True)
    return xc * jax.lax.rsqrt(v + EPS)


def _rb(x):
    return x.astype(jnp.bfloat16).astype(jnp.float32)


def _perm_tile(load_tile, a, p, b21, low):
    a0, a21 = a & 1, a >> 1
    t0 = (((b21 * 2 + 0) * 4 + p) * 4) + a21
    t1 = (((b21 * 2 + 1) * 4 + p) * 4) + a21
    x0, x1 = load_tile(t0), load_tile(t1)
    if a0 == 0:
        return jnp.where(low, x0, pltpu.roll(x1, 4, 0))
    return jnp.where(low, pltpu.roll(x0, 4, 0), x1)


def _kernel(x_ref, xnext_ref, wqkv_hbm, wo_hbm, w1_hbm, w2_hbm, o_ref,
            wqkv_v, wo_v, w1_v, w2_v, t1_scr, wo2_v, q_scr, k_scr, v_scr, oa_scr, xn_scr, sems):
    i = pl.program_id(0)

    def cq(m):
        return pltpu.make_async_copy(wqkv_hbm.at[:, pl.ds(m * D, D)], wqkv_v.at[m], sems.at[m])
    co = pltpu.make_async_copy(wo_hbm, wo_v, sems.at[3])
    c1 = pltpu.make_async_copy(w1_hbm, w1_v, sems.at[4])
    c2 = pltpu.make_async_copy(w2_hbm, w2_v, sems.at[5])

    @pl.when(i == 0)
    def _prep():
        cq(0).start()
        cq(1).start()
        cq(2).start()
        k_scr[0:HALO, :] = jnp.zeros((HALO, D), jnp.float32)
        v_scr[0:HALO, :] = jnp.zeros((HALO, D), jnp.float32)
        xn_scr[...] = _ln(x_ref[...].astype(jnp.float32)).astype(jnp.bfloat16)
        low = jax.lax.broadcasted_iota(jnp.int32, (8, 128), 0) < 4
        for m in range(3):
            cq(m).wait()
            if m == 0:
                co.start()
            if m == 2:
                c1.start()
                c2.start()
            for cb in range(8):
                for rb in range(4):
                    t1_scr[rb, cb * 128:(cb + 1) * 128, :] = pltpu.bitcast(
                        wqkv_v[m, rb * 256:(rb + 1) * 256, cb * 128:(cb + 1) * 128], jnp.uint32).T
            for a in range(8):
                for rb in range(4):
                    tiles = [_perm_tile(lambda t: t1_scr[rb, t * 8:(t + 1) * 8, :], a, p, b21, low)
                             for p in range(4) for b21 in range(4)]
                    g = jnp.concatenate(tiles, axis=0)
                    wqkv_v[m, rb * 256:(rb + 1) * 256, a * 128:(a + 1) * 128] = pltpu.bitcast(g.T, jnp.bfloat16)
        co.wait()
        for cb in range(8):
            for a in range(8):
                for p in range(4):
                    for b2 in range(2):
                        ld = lambda t: wo_v[t * 8:(t + 1) * 8, cb * 128:(cb + 1) * 128].astype(jnp.float32)
                        g = jnp.concatenate(
                            [_perm_tile(ld, a, p, b2 * 2 + b1, low) for b1 in range(2)], axis=0)
                        r0 = a * 128 + p * 32 + b2 * 16
                        wo2_v[r0:r0 + 16, cb * 128:(cb + 1) * 128] = g.astype(jnp.bfloat16)

    xn = xn_scr[...]
    q_scr[...] = _rb(jnp.dot(xn, wqkv_v[0], preferred_element_type=jnp.float32))
    k_scr[HALO:HALO + T, :] = _rb(jnp.dot(xn, wqkv_v[1], preferred_element_type=jnp.float32))
    v_scr[HALO:HALO + T, :] = _rb(jnp.dot(xn, wqkv_v[2], preferred_element_type=jnp.float32))

    lane = jax.lax.broadcasted_iota(jnp.int32, (R, 128), 1)
    even1 = (lane & 1) == 0
    even2 = (lane & 2) == 0
    row0 = i * T
    for c in range(T // R):
        r0 = c * R
        q = q_scr[r0:r0 + R, :]
        logits = []
        ksh = [k_scr[r0 + HALO - 8 - DIL * a: r0 + HALO - DIL * a + R, :] for a in range(4)]
        for w in range(W):
            kw = ksh[w][8:8 + R] if w < 4 else ksh[w - 4][0:R]
            p = q * kw
            s = p[:, 0:128]
            for cb in range(1, 8):
                s = s + p[:, cb * 128:(cb + 1) * 128]
            s = s + jnp.where(even1, pltpu.roll(s, 127, 1), pltpu.roll(s, 1, 1))
            s = s + jnp.where(even2, pltpu.roll(s, 126, 1), pltpu.roll(s, 2, 1))
            s = s * SCALE
            if w > 0 and r0 < DIL * w:
                rows = row0 + r0 + jax.lax.broadcasted_iota(jnp.int32, (R, 128), 0)
                s = jnp.where(rows >= DIL * w, s, -1e9)
            logits.append(s)
        m = logits[0]
        for w in range(1, W):
            m = jnp.maximum(m, logits[w])
        es = [jnp.exp(l - m) for l in logits]
        den = es[0]
        for w in range(1, W):
            den = den + es[w]
        inv = 1.0 / den
        acc = None
        vsh = [v_scr[r0 + HALO - 8 - DIL * a: r0 + HALO - DIL * a + R, :] for a in range(4)]
        for w in range(W):
            a = es[w] * inv
            a8 = jnp.concatenate([a] * 8, axis=1)
            vw = vsh[w][8:8 + R] if w < 4 else vsh[w - 4][0:R]
            acc = a8 * vw if acc is None else acc + a8 * vw
        oa_scr[r0:r0 + R, :] = acc.astype(jnp.bfloat16)

    k_scr[0:HALO, :] = k_scr[T:T + HALO, :]
    v_scr[0:HALO, :] = v_scr[T:T + HALO, :]

    ao = jnp.dot(oa_scr[...], wo2_v[...], preferred_element_type=jnp.float32)
    h = _rb(x_ref[...].astype(jnp.float32) + _rb(ao))
    hn = _ln(h).astype(jnp.bfloat16)
    pl.when(i == 0)(lambda: c1.wait())
    h1 = jnp.maximum(jnp.dot(hn, w1_v[...], preferred_element_type=jnp.float32), 0.0).astype(jnp.bfloat16)
    xn_scr[...] = _ln(xnext_ref[...].astype(jnp.float32)).astype(jnp.bfloat16)
    pl.when(i == 0)(lambda: c2.wait())
    y = jnp.dot(h1, w2_v[...], preferred_element_type=jnp.float32)
    o_ref[...] = (h + _rb(y)).astype(jnp.bfloat16)


@jax.jit
def pallas_sequential_preLN__sliding_local_dilated__dense_activation_relu__prompt_kernel(
    A_x: jax.Array,
    A_wqkv: jax.Array,
    A_wo: jax.Array,
    B_x: jax.Array,
    B_w1: jax.Array,
    B_w2: jax.Array,
):
    x = A_x.reshape(S, D)
    out = pl.pallas_call(
        _kernel,
        grid=(N,),
        in_specs=[
            pl.BlockSpec((T, D), lambda i: (i, 0)),
            pl.BlockSpec((T, D), lambda i: (jnp.minimum(i + 1, N - 1), 0)),
            pl.BlockSpec(memory_space=pl.ANY),
            pl.BlockSpec(memory_space=pl.ANY),
            pl.BlockSpec(memory_space=pl.ANY),
            pl.BlockSpec(memory_space=pl.ANY),
        ],
        out_specs=pl.BlockSpec((T, D), lambda i: (i, 0)),
        out_shape=jax.ShapeDtypeStruct((S, D), jnp.bfloat16),
        scratch_shapes=[
            pltpu.VMEM((3, D, D), jnp.bfloat16),
            pltpu.VMEM((D, D), jnp.bfloat16),
            pltpu.VMEM((D, DFF), jnp.bfloat16),
            pltpu.VMEM((DFF, D), jnp.bfloat16),
            pltpu.VMEM((4, D, 128), jnp.uint32),
            pltpu.VMEM((D, D), jnp.bfloat16),
            pltpu.VMEM((T, D), jnp.float32),
            pltpu.VMEM((T + HALO, D), jnp.float32),
            pltpu.VMEM((T + HALO, D), jnp.float32),
            pltpu.VMEM((T, D), jnp.bfloat16),
            pltpu.VMEM((T, D), jnp.bfloat16),
            pltpu.SemaphoreType.DMA((6,)),
        ],
        compiler_params=pltpu.CompilerParams(
            dimension_semantics=("arbitrary",),
            vmem_limit_bytes=100 * 1024 * 1024,
        ),
    )(x, x, A_wqkv, A_wo, B_w1, B_w2)
    return out.reshape(1, S, D)
```
